```python
import jax
import jax.numpy as jnp

def _softmax(x, axis=-1):
    return jax.nn.softmax(x, axis=axis)
def _gelu(x):
    return jax.nn.gelu(x, approximate=True)
def _silu(x):
    return jax.nn.silu(x)
def _sigmoid(x):
    return jax.nn.sigmoid(x)
def _layernorm(x, axis=-1, eps=1e-5):
    m = jnp.mean(x, axis=axis, keepdims=True)
    v = jnp.var(x, axis=axis, keepdims=True)
    return (x - m) / jnp.sqrt(v + eps)
def _scatter_add(tgt, idx, src, axis=0):
    return tgt.at[idx].add(src)
def _segment_sum(src, seg, n):
    return jax.ops.segment_sum(src, seg, n)
class _Rng:
    def __init__(self, key):
        self._k = key
    def _next(self):
        self._k, sub = jax.random.split(self._k)
        return sub
    def normal(self, shape):
        return jax.random.normal(self._next(), shape, dtype=jnp.bfloat16)
    def randint(self, lo, hi, shape):
        return jax.random.randint(self._next(), shape, lo, hi, dtype=jnp.int32)
    def uniform(self, shape, lo=0.0, hi=1.0):
        return jax.random.uniform(self._next(), shape, jnp.bfloat16, lo, hi)
    def permutation(self, n):
        return jax.random.permutation(self._next(), n)


kernel_name = 'gated_mix__compressed_kv_cla__ssm_conv_h3__prompt'

def setup_inputs():
    _rng = _Rng(jax.random.key(int.from_bytes(__import__("os").urandom(4), "little")))
    _w = (lambda a: (lambda t: t.astype(jnp.bfloat16) if jnp.issubdtype(t.dtype, jnp.floating) else t)(jnp.asarray(a)))
    def _A_setup():
        B, H, Sq, Sk, D, M = 1, 32, 2048, 2048, 128, 1024
        Dc = 4 * D
        return {
            "x": _w((lambda *s: _rng.normal(s) * 0.05)(B, Sq, M)),
            "c_kv": _w((lambda *s: _rng.normal(s) * 0.05)(B, Sk, Dc)),
            "w_q": _w((lambda *s: _rng.normal(s) * 0.05)(M, H, D) * (M ** -0.5)),
            "w_uk": _w((lambda *s: _rng.normal(s) * 0.05)(Dc, H, D) * (Dc ** -0.5)),
            "w_uv": _w((lambda *s: _rng.normal(s) * 0.05)(Dc, H, D) * (Dc ** -0.5)),
            "w_o": _w((lambda *s: _rng.normal(s) * 0.05)(H, D, M) * ((H * D) ** -0.5)),
        }
    _A_in = _A_setup()

    def _B_setup():
        B, S, D = 1, 2048, 1024
        ks = 4
        return {
            "q": _w((lambda *s: _rng.normal(s) * 0.05)(B, S, D)),
            "k": _w((lambda *s: _rng.normal(s) * 0.05)(B, S, D)),
            "v": _w((lambda *s: _rng.normal(s) * 0.05)(B, S, D)),
            "shift_k": _w((lambda *s: _rng.normal(s) * 0.05)(D, ks) * 0.5),
            "ssm_k": _w((lambda *s: _rng.normal(s) * 0.05)(D, S) * (1.0 / S ** 0.5)),
            "ssm_D": _w((lambda *s: _rng.normal(s) * 0.05)(D)),
        }
    _B_in = _B_setup()

    return {
        "A_x": _A_in["x"],
        "A_c_kv": _A_in["c_kv"],
        "A_w_q": _A_in["w_q"],
        "A_w_uk": _A_in["w_uk"],
        "A_w_uv": _A_in["w_uv"],
        "A_w_o": _A_in["w_o"],
        "B_q": _B_in["q"],
        "B_k": _B_in["k"],
        "B_v": _B_in["v"],
        "B_shift_k": _B_in["shift_k"],
        "B_ssm_k": _B_in["ssm_k"],
        "B_ssm_D": _B_in["ssm_D"],
        "gate_w": _w((lambda *s: _rng.normal(s) * 0.05)(1024)),
    }

def reference(A_x, A_c_kv, A_w_q, A_w_uk, A_w_uv, A_w_o, B_q, B_k, B_v, B_shift_k, B_ssm_k, B_ssm_D, gate_w):
    def _A_ref(x, c_kv, w_q, w_uk, w_uv, w_o):
        B, Sq, M = x.shape[0], x.shape[1], x.shape[2]
        Sk = c_kv.shape[1]
        H, D = w_q.shape[1], w_q.shape[2]
        q = jnp.einsum("bqm,mhd->bhqd", x, w_q)
        k = jnp.einsum("bkc,chd->bhkd", c_kv, w_uk)
        v = jnp.einsum("bkc,chd->bhkd", c_kv, w_uv)
        scores = jnp.einsum("bhqd,bhkd->bhqk", q, k) * (D ** -0.5)
        off = Sk - Sq
        qi = jnp.arange(Sq)[:, None]
        kj = jnp.arange(Sk)[None, :]
        cmask = kj <= (qi + off)
        scores = jnp.where(cmask[None, None], scores, -1e9)
        p = _softmax(scores, axis=-1)
        ctx = jnp.einsum("bhqk,bhkd->bhqd", p, v)
        return jnp.einsum("bhqd,hdm->bqm", ctx, w_o)

    def _B_ref(q, k, v, shift_k, ssm_k, ssm_D):
        B, S, D = q.shape
        ks = shift_k.shape[-1]
        k_pad = jnp.pad(k, ((0, 0), (ks - 1, 0), (0, 0)))
        k_shift = jnp.zeros_like(k)
        for t in range(ks):
            k_shift = k_shift + k_pad[:, t:t + S, :] * shift_k[:, ks - 1 - t][None, None, :]
        kv = k_shift * v
        L = 2 * S
        kv_pad = jnp.pad(kv, ((0, 0), (0, S), (0, 0)))
        kf_pad = jnp.pad(ssm_k, ((0, 0), (0, S)))
        kv_f = (lambda x, axes=(-2,-1): jnp.fft.rfft2(x.astype(jnp.float32), axes=axes))(kv_pad[:, None, :, :], axes=(1, 2))
        kf_f = (lambda x, axes=(-2,-1): jnp.fft.rfft2(x.astype(jnp.float32), axes=axes))(kf_pad[:, None, :], axes=(1, 2))
        kf_f = (lambda x, *d: x.transpose(*d))(kf_f, 1, 2, 0)
        y_f = kv_f * kf_f[None, :, :, :]
        y = (lambda x, s, axes=(-2,-1): jnp.fft.irfft2(x, s=s, axes=axes).astype(jnp.bfloat16))(y_f, (1, L), axes=(1, 2))[:, 0, :S, :]
        y = y + kv * ssm_D[None, None, :]
        return q * y

    x = A_x
    g = _sigmoid((x * gate_w).sum(-1, keepdims=True))
    a = _A_ref(x, A_c_kv, A_w_q, A_w_uk, A_w_uv, A_w_o)
    b = _B_ref(x, B_k, B_v, B_shift_k, B_ssm_k, B_ssm_D)
    return g * a + (1 - g) * b
```

```python
import functools
import math

import jax
import jax.numpy as jnp
import numpy as np
import jax.experimental.pallas as pl
import jax.experimental.pallas.tpu as pltpu

S = 2048
M = 1024
DC = 512
H = 32
D = 128
T = 128
NB = S // T
BF = jnp.bfloat16
F32 = jnp.float32


def _dft_consts():
    k = np.arange(T)[:, None] + 0.5
    t = np.arange(T)[None, :]
    ang = 2 * np.pi * k * t / (2 * T)
    fwd = np.concatenate([np.cos(ang), -np.sin(ang)], 0)
    inv = np.concatenate([np.cos(ang).T, -np.sin(ang).T], 1) / T
    return fwd.astype(np.float32), inv.astype(np.float32)


def _kernel(x_hbm, c_hbm, wq_hbm, wk_hbm, wv_hbm, wo_hbm, bk_hbm, bv_hbm, sk_hbm,
            shift_ref, sd_ref, gw_ref, fwd_ref, inv_ref, o_ref,
            x_s, c_s, w_s, wo_s, bk_s, bv_s, sk_s, u_s, h_s, kv_s, b_s,
            q_s, k_s, v_s, ctx_s, sems):
    BQ = 256
    nt = (((1,), (1,)), ((), ()))

    def w_copies(p, slot):
        return [
            pltpu.make_async_copy(wq_hbm.bitcast(jnp.uint32).at[:, p, :],
                                  w_s.at[slot, pl.ds(0, M)], sems.at[6 + slot * 3]),
            pltpu.make_async_copy(wk_hbm.bitcast(jnp.uint32).at[:, p, :],
                                  w_s.at[slot, pl.ds(M, DC)], sems.at[7 + slot * 3]),
            pltpu.make_async_copy(wv_hbm.bitcast(jnp.uint32).at[:, p, :],
                                  w_s.at[slot, pl.ds(M + DC, DC)], sems.at[8 + slot * 3]),
        ]

    cps = [pltpu.make_async_copy(a, b, sems.at[i]) for i, (a, b) in enumerate(
        [(bk_hbm, bk_s), (bv_hbm, bv_s), (sk_hbm, sk_s), (x_hbm, x_s), (c_hbm, c_s),
         (wo_hbm, wo_s)])]
    for cp in cps[:5]:
        cp.start()
    for cp in w_copies(0, 0):
        cp.start()
    cps[5].start()
    for cp in cps[:4]:
        cp.wait()

    fwd = fwd_ref[...]
    inv = inv_ref[...]
    row = jax.lax.broadcasted_iota(jnp.int32, (S, 128), 0)
    sgn = (1 - 2 * (jax.lax.broadcasted_iota(jnp.int32, (T, 128), 0) & 1)).astype(F32)

    def b_chunk(ci, _):
        cs = pl.ds(pl.multiple_of(ci * 128, 128), 128)
        k = bk_s[:, cs].astype(F32)
        sh = shift_ref[:, cs].astype(F32)
        ks = k * sh[0:1]
        for j in range(1, 4):
            ks = ks + jnp.where(row >= j, pltpu.roll(k, j, 0), 0.0) * sh[j:j + 1]
        kv = ks.astype(BF).astype(F32) * bv_s[:, cs].astype(F32)
        kv_s[...] = kv.astype(BF)
        prev = None
        for a in range(NB):
            u_s[a] = jnp.dot(fwd, kv_s[a * T:(a + 1) * T, :], preferred_element_type=F32)
            hh = jax.lax.dot_general(fwd, sk_s[cs, a * T:(a + 1) * T], nt,
                                     preferred_element_type=F32)
            if prev is None:
                h_s[a] = hh
            else:
                h_s[a, :T] = hh[:T] - sgn * prev[T:]
                h_s[a, T:] = hh[T:] + sgn * prev[:T]
            prev = hh
        sd = sd_ref[:, cs].astype(F32)
        for j in range(NB):
            yr = yi = None
            for a in range(j + 1):
                ur, ui = u_s[a, :T], u_s[a, T:]
                hr, hi = h_s[j - a, :T], h_s[j - a, T:]
                r = ur * hr - ui * hi
                i = ur * hi + ui * hr
                yr = r if yr is None else yr + r
                yi = i if yi is None else yi + i
            yy = jnp.concatenate([yr, yi], 0).astype(BF)
            y = jnp.dot(inv, yy, preferred_element_type=F32)
            rs = pl.ds(j * T, T)
            y = y + kv_s[rs, :].astype(F32) * sd
            b_s[rs, cs] = (y * x_s[rs, cs].astype(F32)).astype(BF)
        return None

    jax.lax.fori_loop(0, M // 128, b_chunk, None)

    cps[4].wait()
    qscale = (D ** -0.5) * math.log2(math.e)
    tri = (jax.lax.broadcasted_iota(jnp.int32, (BQ, BQ), 1)
           <= jax.lax.broadcasted_iota(jnp.int32, (BQ, BQ), 0))

    def unpack(w):
        lo = pltpu.bitcast(w << 16, F32).astype(BF)
        hi = pltpu.bitcast(w & jnp.uint32(0xFFFF0000), F32).astype(BF)
        return jnp.concatenate([lo, hi], 1)

    def pair(p, _):
        slot = p % 2

        @pl.when(p + 1 < H // 2)
        def _():
            for cp in w_copies(p + 1, 1 - slot):
                cp.start()
        for cp in w_copies(p, slot):
            cp.wait()
        wq = unpack(w_s[slot, 0:M])
        wkv = jnp.concatenate([unpack(w_s[slot, M:M + DC]), unpack(w_s[slot, M + DC:])], 1)
        for i in range(S // 512):
            rs = pl.ds(i * 512, 512)
            q = (jnp.dot(x_s[rs, :], wq, preferred_element_type=F32) * qscale).astype(BF)
            kv = jnp.dot(c_s[rs, :], wkv, preferred_element_type=F32).astype(BF)
            for e in range(2):
                q_s[e, rs, :] = q[:, e * D:(e + 1) * D]
                k_s[e, rs, :] = kv[:, e * D:(e + 1) * D]
                v_s[e, rs, :] = kv[:, (2 + e) * D:(3 + e) * D]

        def head(e, _):
            for i in range(S // BQ):
                L = (i + 1) * BQ
                rs = pl.ds(i * BQ, BQ)
                s = jax.lax.dot_general(q_s[e, rs, :], k_s[e, 0:L, :], nt,
                                        preferred_element_type=F32)
                sd_ = jnp.where(tri, s[:, L - BQ:], -1e30)
                s = sd_ if i == 0 else jnp.concatenate([s[:, :L - BQ], sd_], 1)
                m = jnp.max(s, axis=1, keepdims=True)
                pe = jnp.exp2(s - m)
                l = jnp.sum(pe, axis=1, keepdims=True)
                o = jnp.dot(pe.astype(BF), v_s[e, 0:L, :], preferred_element_type=F32)
                ctx_s[2 * p + e, rs, :] = (o / l).astype(BF)
            return None

        jax.lax.fori_loop(0, 2, head, None)
        return None

    jax.lax.fori_loop(0, H // 2, pair, None)

    cps[5].wait()
    gw = gw_ref[...].astype(F32)

    def fin(i, _):
        rs = pl.ds(pl.multiple_of(i * 256, 256), 256)
        ctx = jnp.concatenate([ctx_s[h, rs, :] for h in range(H)], 1)
        a = jnp.dot(ctx, wo_s[...], preferred_element_type=F32)
        g = jax.nn.sigmoid(jnp.sum(x_s[rs, :].astype(F32) * gw, axis=1, keepdims=True))
        o_ref[rs, :] = (g * a + (1.0 - g) * b_s[rs, :].astype(F32)).astype(BF)
        return None

    jax.lax.fori_loop(0, S // 256, fin, None)


@jax.jit
def pallas_gated_mix__compressed_kv_cla__ssm_conv_h3__prompt_kernel(
    A_x, A_c_kv, A_w_q, A_w_uk, A_w_uv, A_w_o, B_q, B_k, B_v,
    B_shift_k, B_ssm_k, B_ssm_D, gate_w,
):
    del B_q
    fwd, inv = _dft_consts()
    anyspec = pl.BlockSpec(memory_space=pl.ANY)
    vm = pl.BlockSpec(memory_space=pltpu.VMEM)
    out = pl.pallas_call(
        _kernel,
        in_specs=[anyspec] * 9 + [vm] * 5,
        out_specs=vm,
        out_shape=jax.ShapeDtypeStruct((S, M), BF),
        scratch_shapes=[
            pltpu.VMEM((S, M), BF), pltpu.VMEM((S, DC), BF),
            pltpu.VMEM((2, M + 2 * DC, D), jnp.uint32), pltpu.VMEM((H * D, M), BF),
            pltpu.VMEM((S, M), BF), pltpu.VMEM((S, M), BF), pltpu.VMEM((M, S), BF),
            pltpu.VMEM((NB, 2 * T, 128), F32), pltpu.VMEM((NB, 2 * T, 128), F32),
            pltpu.VMEM((S, 128), BF), pltpu.VMEM((S, M), BF),
            pltpu.VMEM((2, S, D), BF), pltpu.VMEM((2, S, D), BF), pltpu.VMEM((2, S, D), BF),
            pltpu.VMEM((H, S, D), BF),
            pltpu.SemaphoreType.DMA((12,)),
        ],
        compiler_params=pltpu.CompilerParams(vmem_limit_bytes=100 * 1024 * 1024),
    )(A_x[0], A_c_kv[0], A_w_q, A_w_uk, A_w_uv, A_w_o.reshape(H * D, M),
      B_k[0], B_v[0], B_ssm_k, B_shift_k.T, B_ssm_D.reshape(1, M), gate_w.reshape(1, M),
      jnp.asarray(fwd, BF), jnp.asarray(inv, BF))
    return out[None]
```

```python
import functools
import math

import jax
import jax.numpy as jnp
import numpy as np
import jax.experimental.pallas as pl
import jax.experimental.pallas.tpu as pltpu

S = 2048
M = 1024
DC = 512
H = 32
D = 128
T = 128
NB = S // T
BF = jnp.bfloat16
F32 = jnp.float32


def _dft_consts():
    k = np.arange(T)[:, None] + 0.5
    t = np.arange(T)[None, :]
    ang = 2 * np.pi * k * t / (2 * T)
    fwd = np.concatenate([np.cos(ang), -np.sin(ang)], 0)
    inv = np.concatenate([np.cos(ang).T, -np.sin(ang).T], 1) / T
    return fwd.astype(np.float32), inv.astype(np.float32)


def _kernel(x_hbm, c_hbm, wq_hbm, wk_hbm, wv_hbm, wo_hbm, bk_hbm, bv_hbm, sk_hbm,
            shift_ref, sd_ref, gw_ref, fwd_ref, inv_ref, o_ref,
            x_s, c_s, w_s, wo_s, bk_s, bv_s, sk_s, u_s, h_s, kv_s, b_s,
            qkv0, qkv1, ctx_s, sems):
    BQ = 256
    nt = (((1,), (1,)), ((), ()))

    def w_copies(p, slot):
        return [
            pltpu.make_async_copy(wq_hbm.bitcast(jnp.uint32).at[:, p, :],
                                  w_s.at[slot, pl.ds(0, M)], sems.at[6 + slot * 3]),
            pltpu.make_async_copy(wk_hbm.bitcast(jnp.uint32).at[:, p, :],
                                  w_s.at[slot, pl.ds(M, DC)], sems.at[7 + slot * 3]),
            pltpu.make_async_copy(wv_hbm.bitcast(jnp.uint32).at[:, p, :],
                                  w_s.at[slot, pl.ds(M + DC, DC)], sems.at[8 + slot * 3]),
        ]

    cps = [pltpu.make_async_copy(a, b, sems.at[i]) for i, (a, b) in enumerate(
        [(bk_hbm, bk_s), (bv_hbm, bv_s), (sk_hbm, sk_s), (x_hbm, x_s), (c_hbm, c_s),
         (wo_hbm, wo_s)])]
    for cp in [cps[3], cps[4]] + w_copies(0, 0) + w_copies(1, 1) + cps[:3] + [cps[5]]:
        cp.start()

    fwd = fwd_ref[...]
    inv = inv_ref[...]
    row = jax.lax.broadcasted_iota(jnp.int32, (S, 128), 0)
    sgn = (1 - 2 * (jax.lax.broadcasted_iota(jnp.int32, (T, 128), 0) & 1)).astype(F32)

    def b_chunk(ci):
        cs = pl.ds(pl.multiple_of(ci * 128, 128), 128)
        k = bk_s[:, cs].astype(F32)
        sh = shift_ref[:, cs].astype(F32)
        ks = k * sh[0:1]
        for j in range(1, 4):
            ks = ks + jnp.where(row >= j, pltpu.roll(k, j, 0), 0.0) * sh[j:j + 1]
        kv = ks.astype(BF).astype(F32) * bv_s[:, cs].astype(F32)
        kv_s[...] = kv.astype(BF)
        yield
        prev = None
        for a in range(NB):
            u_s[a] = jnp.dot(fwd, kv_s[a * T:(a + 1) * T, :], preferred_element_type=F32)
            hh = jax.lax.dot_general(fwd, sk_s[cs, a * T:(a + 1) * T], nt,
                                     preferred_element_type=F32)
            if prev is None:
                h_s[a] = hh
            else:
                h_s[a, :T] = hh[:T] - sgn * prev[T:]
                h_s[a, T:] = hh[T:] + sgn * prev[:T]
            prev = hh
            if a % 8 == 7:
                yield
        sd = sd_ref[:, cs].astype(F32)
        for j in range(NB):
            yr = yi = None
            for a in range(j + 1):
                ur, ui = u_s[a, :T], u_s[a, T:]
                hr, hi = h_s[j - a, :T], h_s[j - a, T:]
                r = ur * hr - ui * hi
                i = ur * hi + ui * hr
                yr = r if yr is None else yr + r
                yi = i if yi is None else yi + i
            yy = jnp.concatenate([yr, yi], 0).astype(BF)
            y = jnp.dot(inv, yy, preferred_element_type=F32)
            rs = pl.ds(j * T, T)
            y = y + kv_s[rs, :].astype(F32) * sd
            b_s[rs, cs] = (y * x_s[rs, cs].astype(F32)).astype(BF)
            if j >= 3:
                yield

    cps[3].wait()
    cps[4].wait()
    qscale = (D ** -0.5) * math.log2(math.e)
    tri = (jax.lax.broadcasted_iota(jnp.int32, (BQ, BQ), 1)
           <= jax.lax.broadcasted_iota(jnp.int32, (BQ, BQ), 0))

    def unpack(w):
        lo = pltpu.bitcast(w << 16, F32).astype(BF)
        hi = pltpu.bitcast(w & jnp.uint32(0xFFFF0000), F32).astype(BF)
        return jnp.concatenate([lo, hi], 1)

    def get_w(p, slot):
        for cp in w_copies(p, slot):
            cp.wait()
        wq = unpack(w_s[slot, 0:M])
        wkv = jnp.concatenate([unpack(w_s[slot, M:M + DC]), unpack(w_s[slot, M + DC:])], 1)
        return wq, wkv

    def proj(w, dst, i):
        rs = pl.ds(i * BQ, BQ)
        q = (jnp.dot(x_s[rs, :], w[0], preferred_element_type=F32) * qscale).astype(BF)
        kv = jnp.dot(c_s[rs, :], w[1], preferred_element_type=F32).astype(BF)
        for e in range(2):
            dst[e, rs, :] = q[:, e * D:(e + 1) * D]
        for e in range(4):
            dst[2 + e, rs, :] = kv[:, e * D:(e + 1) * D]

    def attn(src, e, h, i):
        L = (i + 1) * BQ
        rs = pl.ds(i * BQ, BQ)
        s = jax.lax.dot_general(src[e, rs, :], src[2 + e, 0:L, :], nt,
                                preferred_element_type=F32)
        sd_ = jnp.where(tri, s[:, L - BQ:], -1e30)
        s = sd_ if i == 0 else jnp.concatenate([s[:, :L - BQ], sd_], 1)
        m = jnp.max(s, axis=1, keepdims=True)
        pe = jnp.exp2(s - m)
        l = jnp.sum(pe, axis=1, keepdims=True)
        o = jnp.dot(pe.astype(BF), src[4 + e, 0:L, :], preferred_element_type=F32)
        ctx_s[h, rs, :] = (o / l).astype(BF)

    w0 = get_w(0, 0)
    for i in range(S // BQ):
        proj(w0, qkv0, i)
    for cp in cps[:3]:
        cp.wait()

    def quad(g, last):
        bg = b_chunk(g)
        for half, (src, dst) in enumerate([(qkv0, qkv1), (qkv1, qkv0)]):
            p = 2 * g + half
            do_proj = not (last and half == 1)
            if do_proj:
                w = get_w(p + 1, 1 - half)
            if not last:
                for cp in w_copies(p + 2, half):
                    cp.start()
            for i in range(S // BQ):
                if do_proj:
                    proj(w, dst, i)
                next(bg, None)
                for e in range(2):
                    attn(src, e, 2 * p + e, i)

    jax.lax.fori_loop(0, H // 4 - 1, lambda g, _: quad(g, False), None)
    quad(H // 4 - 1, True)

    cps[5].wait()
    gw = gw_ref[...].astype(F32)

    def fin(i, _):
        rs = pl.ds(pl.multiple_of(i * 256, 256), 256)
        ctx = jnp.concatenate([ctx_s[h, rs, :] for h in range(H)], 1)
        a = jnp.dot(ctx, wo_s[...], preferred_element_type=F32)
        g = jax.nn.sigmoid(jnp.sum(x_s[rs, :].astype(F32) * gw, axis=1, keepdims=True))
        o_ref[rs, :] = (g * a + (1.0 - g) * b_s[rs, :].astype(F32)).astype(BF)
        return None

    jax.lax.fori_loop(0, S // 256, fin, None)


@jax.jit
def pallas_gated_mix__compressed_kv_cla__ssm_conv_h3__prompt_kernel(
    A_x, A_c_kv, A_w_q, A_w_uk, A_w_uv, A_w_o, B_q, B_k, B_v,
    B_shift_k, B_ssm_k, B_ssm_D, gate_w,
):
    del B_q
    fwd, inv = _dft_consts()
    anyspec = pl.BlockSpec(memory_space=pl.ANY)
    vm = pl.BlockSpec(memory_space=pltpu.VMEM)
    out = pl.pallas_call(
        _kernel,
        in_specs=[anyspec] * 9 + [vm] * 5,
        out_specs=vm,
        out_shape=jax.ShapeDtypeStruct((S, M), BF),
        scratch_shapes=[
            pltpu.VMEM((S, M), BF), pltpu.VMEM((S, DC), BF),
            pltpu.VMEM((2, M + 2 * DC, D), jnp.uint32), pltpu.VMEM((H * D, M), BF),
            pltpu.VMEM((S, M), BF), pltpu.VMEM((S, M), BF), pltpu.VMEM((M, S), BF),
            pltpu.VMEM((NB, 2 * T, 128), F32), pltpu.VMEM((NB, 2 * T, 128), F32),
            pltpu.VMEM((S, 128), BF), pltpu.VMEM((S, M), BF),
            pltpu.VMEM((6, S, D), BF), pltpu.VMEM((6, S, D), BF),
            pltpu.VMEM((H, S, D), BF),
            pltpu.SemaphoreType.DMA((12,)),
        ],
        compiler_params=pltpu.CompilerParams(vmem_limit_bytes=120 * 1024 * 1024),
    )(A_x[0], A_c_kv[0], A_w_q, A_w_uk, A_w_uv, A_w_o.reshape(H * D, M),
      B_k[0], B_v[0], B_ssm_k, B_shift_k.T, B_ssm_D.reshape(1, M), gate_w.reshape(1, M),
      jnp.asarray(fwd, BF), jnp.asarray(inv, BF))
    return out[None]
```

```python
import functools
import math

import jax
import jax.numpy as jnp
import numpy as np
import jax.experimental.pallas as pl
import jax.experimental.pallas.tpu as pltpu

S = 2048
M = 1024
DC = 512
H = 32
D = 128
T = 128
NB = S // T
BF = jnp.bfloat16
F32 = jnp.float32


def _dft_consts():
    k = np.arange(T)[:, None] + 0.5
    t = np.arange(T)[None, :]
    ang = 2 * np.pi * k * t / (2 * T)
    fwd = np.concatenate([np.cos(ang), -np.sin(ang)], 0)
    inv = np.concatenate([np.cos(ang).T, -np.sin(ang).T], 1) / T
    return fwd.astype(np.float32), inv.astype(np.float32)


def _kernel(x_hbm, c_hbm, wq_hbm, wk_hbm, wv_hbm, wo_hbm, bk_hbm, bv_hbm, sk_hbm,
            shift_ref, sd_ref, gw_ref, fwd_ref, inv_ref, o_ref,
            x_s, c_s, w_s, wo_s, bk_s, bv_s, sk_s, u_s, h_s, kv_s, b_s,
            qkv0, qkv1, ctx_s, sems):
    BQ = 256
    nt = (((1,), (1,)), ((), ()))

    def w_copies(p, slot):
        return [
            pltpu.make_async_copy(wq_hbm.bitcast(jnp.uint32).at[:, p, :],
                                  w_s.at[slot, pl.ds(0, M)], sems.at[6 + slot * 3]),
            pltpu.make_async_copy(wk_hbm.bitcast(jnp.uint32).at[:, p, :],
                                  w_s.at[slot, pl.ds(M, DC)], sems.at[7 + slot * 3]),
            pltpu.make_async_copy(wv_hbm.bitcast(jnp.uint32).at[:, p, :],
                                  w_s.at[slot, pl.ds(M + DC, DC)], sems.at[8 + slot * 3]),
        ]

    cps = [pltpu.make_async_copy(a, b, sems.at[i]) for i, (a, b) in enumerate(
        [(bk_hbm, bk_s), (bv_hbm, bv_s), (sk_hbm, sk_s), (x_hbm, x_s), (c_hbm, c_s),
         (wo_hbm, wo_s)])]
    for cp in [cps[3], cps[4]] + w_copies(0, 0) + w_copies(1, 1) + cps[:3] + [cps[5]]:
        cp.start()

    fwd = fwd_ref[...]
    inv = inv_ref[...]
    row = jax.lax.broadcasted_iota(jnp.int32, (S, 128), 0)
    sgn = (1 - 2 * (jax.lax.broadcasted_iota(jnp.int32, (T, 128), 0) & 1)).astype(F32)

    def b_chunk(ci):
        cs = pl.ds(pl.multiple_of(ci * 128, 128), 128)
        k = bk_s[:, cs].astype(F32)
        sh = shift_ref[:, cs].astype(F32)
        ks = k * sh[0:1]
        for j in range(1, 4):
            ks = ks + jnp.where(row >= j, pltpu.roll(k, j, 0), 0.0) * sh[j:j + 1]
        kv = ks.astype(BF).astype(F32) * bv_s[:, cs].astype(F32)
        kv_s[...] = kv.astype(BF)
        yield
        prev = None
        for a in range(NB):
            u_s[a] = jnp.dot(fwd, kv_s[a * T:(a + 1) * T, :], preferred_element_type=F32)
            hh = jax.lax.dot_general(fwd, sk_s[cs, a * T:(a + 1) * T], nt,
                                     preferred_element_type=F32)
            if prev is None:
                h_s[a] = hh
            else:
                h_s[a, :T] = hh[:T] - sgn * prev[T:]
                h_s[a, T:] = hh[T:] + sgn * prev[:T]
            prev = hh
            if a % 8 == 7:
                yield
        sd = sd_ref[:, cs].astype(F32)
        for j in range(NB):
            yr = yi = None
            for a in range(j + 1):
                ur, ui = u_s[a, :T], u_s[a, T:]
                hr, hi = h_s[j - a, :T], h_s[j - a, T:]
                r = ur * hr - ui * hi
                i = ur * hi + ui * hr
                yr = r if yr is None else yr + r
                yi = i if yi is None else yi + i
            yy = jnp.concatenate([yr, yi], 0).astype(BF)
            y = jnp.dot(inv, yy, preferred_element_type=F32)
            rs = pl.ds(j * T, T)
            y = y + kv_s[rs, :].astype(F32) * sd
            b_s[rs, cs] = (y * x_s[rs, cs].astype(F32)).astype(BF)
            if j >= 3:
                yield

    cps[3].wait()
    cps[4].wait()
    qscale = (D ** -0.5) * math.log2(math.e)
    tri = (jax.lax.broadcasted_iota(jnp.int32, (BQ, BQ), 1)
           <= jax.lax.broadcasted_iota(jnp.int32, (BQ, BQ), 0))

    def unpack(w):
        lo = pltpu.bitcast(w << 16, F32).astype(BF)
        hi = pltpu.bitcast(w & jnp.uint32(0xFFFF0000), F32).astype(BF)
        return jnp.concatenate([lo, hi], 1)

    def get_w(p, slot):
        for cp in w_copies(p, slot):
            cp.wait()
        wq = unpack(w_s[slot, 0:M])
        wkv = jnp.concatenate([unpack(w_s[slot, M:M + DC]), unpack(w_s[slot, M + DC:])], 1)
        return wq, wkv

    def proj(w, dst, i):
        rs = pl.ds(i * BQ, BQ)
        q = (jnp.dot(x_s[rs, :], w[0], preferred_element_type=F32) * qscale).astype(BF)
        kv = jnp.dot(c_s[rs, :], w[1], preferred_element_type=F32).astype(BF)
        for e in range(2):
            dst[e, rs, :] = q[:, e * D:(e + 1) * D]
        for e in range(4):
            dst[2 + e, rs, :] = kv[:, e * D:(e + 1) * D]

    def attn(src, e, h, i):
        L = (i + 1) * BQ
        rs = pl.ds(i * BQ, BQ)
        s = jax.lax.dot_general(src[e, rs, :], src[2 + e, 0:L, :], nt,
                                preferred_element_type=F32)
        sd_ = jnp.where(tri, s[:, L - BQ:], -1e30)
        s = sd_ if i == 0 else jnp.concatenate([s[:, :L - BQ], sd_], 1)
        m = jnp.max(s, axis=1, keepdims=True)
        yield
        pe = jnp.exp2(s - m)
        l = jnp.sum(pe, axis=1, keepdims=True)
        o = jnp.dot(pe.astype(BF), src[4 + e, 0:L, :], preferred_element_type=F32)
        ctx_s[h, rs, :] = (o / l).astype(BF)

    w0 = get_w(0, 0)
    for i in range(S // BQ):
        proj(w0, qkv0, i)
    for cp in cps[:3]:
        cp.wait()

    def quad(g, last):
        bg = b_chunk(g)
        for half, (src, dst) in enumerate([(qkv0, qkv1), (qkv1, qkv0)]):
            p = 2 * g + half
            do_proj = not (last and half == 1)
            if do_proj:
                w = get_w(p + 1, 1 - half)
            if not last:
                for cp in w_copies(p + 2, half):
                    cp.start()
            for i in range(S // BQ):
                gs = [attn(src, e, 2 * p + e, i) for e in range(2)]
                for a_ in gs:
                    next(a_)
                if do_proj:
                    proj(w, dst, i)
                next(bg, None)
                for a_ in gs:
                    next(a_, None)

    jax.lax.fori_loop(0, H // 4 - 1, lambda g, _: quad(g, False), None)
    quad(H // 4 - 1, True)

    cps[5].wait()
    gw = gw_ref[...].astype(F32)

    def fin(i, _):
        rs = pl.ds(pl.multiple_of(i * 256, 256), 256)
        ctx = jnp.concatenate([ctx_s[h, rs, :] for h in range(H)], 1)
        a = jnp.dot(ctx, wo_s[...], preferred_element_type=F32)
        g = jax.nn.sigmoid(jnp.sum(x_s[rs, :].astype(F32) * gw, axis=1, keepdims=True))
        o_ref[rs, :] = (g * a + (1.0 - g) * b_s[rs, :].astype(F32)).astype(BF)
        return None

    jax.lax.fori_loop(0, S // 256, fin, None)


@jax.jit
def pallas_gated_mix__compressed_kv_cla__ssm_conv_h3__prompt_kernel(
    A_x, A_c_kv, A_w_q, A_w_uk, A_w_uv, A_w_o, B_q, B_k, B_v,
    B_shift_k, B_ssm_k, B_ssm_D, gate_w,
):
    del B_q
    fwd, inv = _dft_consts()
    anyspec = pl.BlockSpec(memory_space=pl.ANY)
    vm = pl.BlockSpec(memory_space=pltpu.VMEM)
    out = pl.pallas_call(
        _kernel,
        in_specs=[anyspec] * 9 + [vm] * 5,
        out_specs=vm,
        out_shape=jax.ShapeDtypeStruct((S, M), BF),
        scratch_shapes=[
            pltpu.VMEM((S, M), BF), pltpu.VMEM((S, DC), BF),
            pltpu.VMEM((2, M + 2 * DC, D), jnp.uint32), pltpu.VMEM((H * D, M), BF),
            pltpu.VMEM((S, M), BF), pltpu.VMEM((S, M), BF), pltpu.VMEM((M, S), BF),
            pltpu.VMEM((NB, 2 * T, 128), F32), pltpu.VMEM((NB, 2 * T, 128), F32),
            pltpu.VMEM((S, 128), BF), pltpu.VMEM((S, M), BF),
            pltpu.VMEM((6, S, D), BF), pltpu.VMEM((6, S, D), BF),
            pltpu.VMEM((H, S, D), BF),
            pltpu.SemaphoreType.DMA((12,)),
        ],
        compiler_params=pltpu.CompilerParams(vmem_limit_bytes=120 * 1024 * 1024),
    )(A_x[0], A_c_kv[0], A_w_q, A_w_uk, A_w_uv, A_w_o.reshape(H * D, M),
      B_k[0], B_v[0], B_ssm_k, B_shift_k.T, B_ssm_D.reshape(1, M), gate_w.reshape(1, M),
      jnp.asarray(fwd, BF), jnp.asarray(inv, BF))
    return out[None]
```
